```python
import jax
import jax.numpy as jnp

def _softmax(x, axis=-1):
    return jax.nn.softmax(x, axis=axis)
def _gelu(x):
    return jax.nn.gelu(x, approximate=True)
def _silu(x):
    return jax.nn.silu(x)
def _sigmoid(x):
    return jax.nn.sigmoid(x)
def _layernorm(x, axis=-1, eps=1e-5):
    m = jnp.mean(x, axis=axis, keepdims=True)
    v = jnp.var(x, axis=axis, keepdims=True)
    return (x - m) / jnp.sqrt(v + eps)
def _scatter_add(tgt, idx, src, axis=0):
    return tgt.at[idx].add(src)
def _segment_sum(src, seg, n):
    return jax.ops.segment_sum(src, seg, n)
class _Rng:
    def __init__(self, key):
        self._k = key
    def _next(self):
        self._k, sub = jax.random.split(self._k)
        return sub
    def normal(self, shape):
        return jax.random.normal(self._next(), shape, dtype=jnp.bfloat16)
    def randint(self, lo, hi, shape):
        return jax.random.randint(self._next(), shape, lo, hi, dtype=jnp.int32)
    def uniform(self, shape, lo=0.0, hi=1.0):
        return jax.random.uniform(self._next(), shape, jnp.bfloat16, lo, hi)
    def permutation(self, n):
        return jax.random.permutation(self._next(), n)


kernel_name = 'gated_mix__mha_block_cached__compressed_kv_cla__decode'

def setup_inputs():
    _rng = _Rng(jax.random.key(int.from_bytes(__import__("os").urandom(4), "little")))
    _w = (lambda a: (lambda t: t.astype(jnp.bfloat16) if jnp.issubdtype(t.dtype, jnp.floating) else t)(jnp.asarray(a)))
    def _A_setup():
        B, Sq, D = 2, 1, 512
        H, Sk, Dh = 32, 8192, 128
        return {
            "x": _w((lambda *s: _rng.normal(s) * 0.05)(B, Sq, D)),
            "k_cache": _w((lambda *s: _rng.normal(s) * 0.05)(B, H, Sk, Dh)),
            "v_cache": _w((lambda *s: _rng.normal(s) * 0.05)(B, H, Sk, Dh)),
            "wq": _w((lambda *s: _rng.normal(s) * 0.05)(D, H * Dh) * (D ** -0.5)),
            "wo": _w((lambda *s: _rng.normal(s) * 0.05)(H * Dh, D) * ((H * Dh) ** -0.5)),
        }
    _A_in = _A_setup()

    def _B_setup():
        B, H, Sq, Sk, D, M = 2, 32, 1, 8192, 128, 512
        Dc = 4 * D
        return {
            "x": _w((lambda *s: _rng.normal(s) * 0.05)(B, Sq, M)),
            "c_kv": _w((lambda *s: _rng.normal(s) * 0.05)(B, Sk, Dc)),
            "w_q": _w((lambda *s: _rng.normal(s) * 0.05)(M, H, D) * (M ** -0.5)),
            "w_uk": _w((lambda *s: _rng.normal(s) * 0.05)(Dc, H, D) * (Dc ** -0.5)),
            "w_uv": _w((lambda *s: _rng.normal(s) * 0.05)(Dc, H, D) * (Dc ** -0.5)),
            "w_o": _w((lambda *s: _rng.normal(s) * 0.05)(H, D, M) * ((H * D) ** -0.5)),
        }
    _B_in = _B_setup()

    return {
        "A_x": _A_in["x"],
        "A_k_cache": _A_in["k_cache"],
        "A_v_cache": _A_in["v_cache"],
        "A_wq": _A_in["wq"],
        "A_wo": _A_in["wo"],
        "B_x": _B_in["x"],
        "B_c_kv": _B_in["c_kv"],
        "B_w_q": _B_in["w_q"],
        "B_w_uk": _B_in["w_uk"],
        "B_w_uv": _B_in["w_uv"],
        "B_w_o": _B_in["w_o"],
        "gate_w": _w((lambda *s: _rng.normal(s) * 0.05)(512)),
    }

def reference(A_x, A_k_cache, A_v_cache, A_wq, A_wo, B_x, B_c_kv, B_w_q, B_w_uk, B_w_uv, B_w_o, gate_w):
    def _A_ref(x, k_cache, v_cache, wq, wo):
        B, Sq, D = x.shape
        H, Dh = 32, 128
        q = (lambda x, *d: x.transpose(*d))((x @ wq).reshape(B, Sq, H, Dh), 0, 2, 1, 3)
        scores = jnp.einsum("bhqd,bhkd->bhqk", q, k_cache) * (Dh ** -0.5)
        p = _softmax(scores, axis=-1)
        o = jnp.einsum("bhqk,bhkd->bhqd", p, v_cache)
        return (lambda x, *d: x.transpose(*d))(o, 0, 2, 1, 3).reshape(B, Sq, H * Dh) @ wo

    def _B_ref(x, c_kv, w_q, w_uk, w_uv, w_o):
        B, Sq, M = x.shape[0], x.shape[1], x.shape[2]
        Sk = c_kv.shape[1]
        H, D = w_q.shape[1], w_q.shape[2]
        q = jnp.einsum("bqm,mhd->bhqd", x, w_q)
        k = jnp.einsum("bkc,chd->bhkd", c_kv, w_uk)
        v = jnp.einsum("bkc,chd->bhkd", c_kv, w_uv)
        scores = jnp.einsum("bhqd,bhkd->bhqk", q, k) * (D ** -0.5)
        off = Sk - Sq
        qi = jnp.arange(Sq)[:, None]
        kj = jnp.arange(Sk)[None, :]
        cmask = kj <= (qi + off)
        scores = jnp.where(cmask[None, None], scores, -1e9)
        p = _softmax(scores, axis=-1)
        ctx = jnp.einsum("bhqk,bhkd->bhqd", p, v)
        return jnp.einsum("bhqd,hdm->bqm", ctx, w_o)

    x = A_x
    g = _sigmoid((x * gate_w).sum(-1, keepdims=True))
    a = _A_ref(x, A_k_cache, A_v_cache, A_wq, A_wo)
    b = _B_ref(x, B_c_kv, B_w_q, B_w_uk, B_w_uv, B_w_o)
    return g * a + (1 - g) * b
```

```python
import jax
import jax.numpy as jnp
import numpy as np
from jax.experimental import pallas as pl
from jax.experimental.pallas import tpu as pltpu

_B = 2
_H = 32
_SK = 8192
_DH = 128
_D = 512
_NBUF = 8
_F32 = jnp.float32
_BF16 = jnp.bfloat16
_NT = (((1,), (1,)), ((), ()))
_SCALE = float(_DH) ** -0.5


def _iota(shape, dim):
    return jax.lax.broadcasted_iota(jnp.int32, shape, dim)


def _kernel(
    x_hbm, k_hbm, v_hbm, wq_hbm, wo_hbm,
    ckv_hbm, wbq_hbm, wuk_hbm, wuv_hbm, wbo_hbm, gate_hbm,
    out_ref,
    x_buf, gate_buf, wq_buf, wo_buf, wbq_buf, wuk_buf, wuv_buf, wbo_buf,
    ckv_buf, k_buf, v_buf, e_buf, q_buf,
    w_sems, c_sems, k_sems, v_sems,
):
    BH = _B * _H

    def w_copy(idx, src, dst):
        return pltpu.make_async_copy(src, dst, w_sems.at[idx])

    cp_x = w_copy(0, x_hbm, x_buf)
    cp_gate = w_copy(1, gate_hbm, gate_buf)
    cp_wq = w_copy(2, wq_hbm, wq_buf)
    cp_wbq = w_copy(3, wbq_hbm, wbq_buf)
    cp_wuk = w_copy(4, wuk_hbm, wuk_buf)
    cp_wuv = w_copy(5, wuv_hbm, wuv_buf)
    cp_wbo = w_copy(6, wbo_hbm, wbo_buf)
    cp_wo = w_copy(7, wo_hbm, wo_buf)

    def c_copy(b):
        return pltpu.make_async_copy(ckv_hbm.at[b], ckv_buf.at[b], c_sems.at[b])

    def k_copy(i, slot):
        return pltpu.make_async_copy(k_hbm.at[i], k_buf.at[slot], k_sems.at[slot])

    def v_copy(i, slot):
        return pltpu.make_async_copy(v_hbm.at[i], v_buf.at[slot], v_sems.at[slot])

    cp_x.start()
    cp_gate.start()
    cp_wbq.start()
    cp_wuk.start()
    cp_wq.start()
    c_copy(0).start()
    c_copy(1).start()
    cp_wuv.start()
    cp_wbo.start()
    cp_wo.start()
    for i in range(_NBUF):
        k_copy(i, i).start()
        v_copy(i, i).start()

    for j in range(8):
        shp = (_DH, 512)
        col = _iota(shp, 1) + j * 512
        e_buf[:, j * 512:(j + 1) * 512] = jnp.where(
            (col >> 5) == _iota(shp, 0), 1.0, 0.0).astype(_BF16)

    diag = (_iota((BH, 4096), 0) & 31) == (_iota((BH, 4096), 1) & 31)
    row8 = _iota((8, _D), 0)

    cp_x.wait()
    x2 = x_buf[...].astype(_F32)
    x8 = jnp.where(row8 == 0, x2[0:1, :], jnp.where(row8 == 1, x2[1:2, :], 0.0))
    x8 = x8.astype(_BF16)

    cp_wbq.wait()
    q_b = jnp.zeros((BH, _DH), _F32)
    for t in range(4):
        xr = jnp.dot(x8[:, t * 128:(t + 1) * 128], e_buf[...],
                     preferred_element_type=_F32)
        xr = jnp.concatenate(
            [jnp.broadcast_to(xr[0:1, :], (_H, 4096)),
             jnp.broadcast_to(xr[1:2, :], (_H, 4096))], axis=0)
        lhs = jnp.where(diag, xr, 0.0).astype(_BF16)
        q_b = q_b + jnp.dot(lhs, wbq_buf[t * 4096:(t + 1) * 4096, :],
                            preferred_element_type=_F32)
    q_b = q_b.astype(_BF16)

    cp_wuk.wait()
    q_abs = []
    for t in range(4):
        r = jax.lax.dot_general(q_b, wuk_buf[t * 4096:(t + 1) * 4096, :], _NT,
                                preferred_element_type=_F32)
        r = jnp.where(diag, r, 0.0).astype(_BF16)
        q_abs.append(jax.lax.dot_general(r, e_buf[...], _NT,
                                         preferred_element_type=_F32))
    q_abs = jnp.concatenate(q_abs, axis=1).astype(_BF16)

    cp_wq.wait()
    q_a = jnp.dot(x8, wq_buf[...], preferred_element_type=_F32)
    q_a = q_a.astype(_BF16)
    for h in range(_H):
        q_buf[h] = q_a[:, h * _DH:(h + 1) * _DH]

    ctx_c = []
    for b in range(_B):
        c_copy(b).wait()
        qb = q_abs[b * _H:(b + 1) * _H, :]
        s = jax.lax.dot_general(qb, ckv_buf[b], _NT,
                                preferred_element_type=_F32) * _SCALE
        m = jnp.max(s, axis=-1, keepdims=True)
        p = jnp.exp(s - m)
        l = jnp.sum(p, axis=-1, keepdims=True)
        cc = jnp.dot(p.astype(_BF16), ckv_buf[b], preferred_element_type=_F32)
        ctx_c.append(cc / l)
    ctx_c = jnp.concatenate(ctx_c, axis=0).astype(_BF16)

    cp_wuv.wait()
    ctx = jnp.zeros((BH, _DH), _F32)
    for t in range(4):
        xr = jnp.dot(ctx_c[:, t * 128:(t + 1) * 128], e_buf[...],
                     preferred_element_type=_F32)
        lhs = jnp.where(diag, xr, 0.0).astype(_BF16)
        ctx = ctx + jnp.dot(lhs, wuv_buf[t * 4096:(t + 1) * 4096, :],
                            preferred_element_type=_F32)
    ctx = ctx.astype(_BF16)

    cp_wbo.wait()
    blk = (_iota((BH, 4096), 0) & 31) == (_iota((BH, 4096), 1) >> 7)
    lhs = jnp.where(blk, jnp.concatenate([ctx] * _H, axis=1), 0.0).astype(_BF16)
    t_b = jnp.dot(lhs, wbo_buf[...], preferred_element_type=_F32)
    ob0 = jnp.sum(t_b[0:_H, :], axis=0, keepdims=True)
    ob1 = jnp.sum(t_b[_H:BH, :], axis=0, keepdims=True)
    out_b = jnp.where(row8 == 0, ob0, jnp.where(row8 == 1, ob1, 0.0))

    cp_gate.wait()
    gw = gate_buf[...].astype(_F32)
    g = jax.nn.sigmoid(jnp.sum(x8.astype(_F32) * gw, axis=-1, keepdims=True))

    cp_wo.wait()
    row_o = _iota((8, _DH), 0)

    def body(i, acc):
        slot = i % _NBUF
        b = i // _H
        h = i % _H
        q = q_buf[h]
        k_copy(i, slot).wait()
        s = jax.lax.dot_general(q, k_buf[slot], _NT,
                                preferred_element_type=_F32) * _SCALE
        m = jnp.max(s, axis=-1, keepdims=True)
        p = jnp.exp(s - m)
        l = jnp.sum(p, axis=-1, keepdims=True)
        v_copy(i, slot).wait()
        o = jnp.dot(p.astype(_BF16), v_buf[slot], preferred_element_type=_F32)

        @pl.when(i + _NBUF < BH)
        def _():
            k_copy(i + _NBUF, slot).start()
            v_copy(i + _NBUF, slot).start()

        o = jnp.where(row_o == b, o / l, 0.0).astype(_BF16)
        wo_h = wo_buf[pl.ds(pl.multiple_of(h * _DH, _DH), _DH), :]
        return acc + jnp.dot(o, wo_h, preferred_element_type=_F32)

    out_a = jax.lax.fori_loop(0, BH, body, jnp.zeros((8, _D), _F32))

    res = g * out_a + (1.0 - g) * out_b
    out_ref[...] = res[0:_B, :].astype(out_ref.dtype)


@jax.jit
def pallas_gated_mix__mha_block_cached__compressed_kv_cla__decode_kernel(
    A_x: jax.Array,
    A_k_cache: jax.Array,
    A_v_cache: jax.Array,
    A_wq: jax.Array,
    A_wo: jax.Array,
    B_x: jax.Array,
    B_c_kv: jax.Array,
    B_w_q: jax.Array,
    B_w_uk: jax.Array,
    B_w_uv: jax.Array,
    B_w_o: jax.Array,
    gate_w: jax.Array,
):
    del B_x
    out_dtype = A_x.dtype
    any_spec = pl.BlockSpec(memory_space=pl.ANY)
    out = pl.pallas_call(
        _kernel,
        out_shape=jax.ShapeDtypeStruct((_B, _D), out_dtype),
        in_specs=[any_spec] * 11,
        out_specs=pl.BlockSpec(memory_space=pltpu.VMEM),
        scratch_shapes=[
            pltpu.VMEM((_B, _D), _BF16),
            pltpu.VMEM((1, _D), _BF16),
            pltpu.VMEM((_D, _H * _DH), _BF16),
            pltpu.VMEM((_H * _DH, _D), _BF16),
            pltpu.VMEM((_D * _H, _DH), _BF16),
            pltpu.VMEM((_D * _H, _DH), _BF16),
            pltpu.VMEM((_D * _H, _DH), _BF16),
            pltpu.VMEM((_H * _DH, _D), _BF16),
            pltpu.VMEM((_B, _SK, _D), _BF16),
            pltpu.VMEM((_NBUF, _SK, _DH), _BF16),
            pltpu.VMEM((_NBUF, _SK, _DH), _BF16),
            pltpu.VMEM((_DH, _H * _DH), _BF16),
            pltpu.VMEM((_H, 8, _DH), _BF16),
            pltpu.SemaphoreType.DMA((8,)),
            pltpu.SemaphoreType.DMA((_B,)),
            pltpu.SemaphoreType.DMA((_NBUF,)),
            pltpu.SemaphoreType.DMA((_NBUF,)),
        ],
        compiler_params=pltpu.CompilerParams(
            vmem_limit_bytes=110 * 1024 * 1024,
        ),
    )(
        A_x.reshape(_B, _D),
        A_k_cache.reshape(_B * _H, _SK, _DH),
        A_v_cache.reshape(_B * _H, _SK, _DH),
        A_wq,
        A_wo,
        B_c_kv,
        B_w_q.reshape(_D * _H, _DH),
        B_w_uk.reshape(_D * _H, _DH),
        B_w_uv.reshape(_D * _H, _DH),
        B_w_o.reshape(_H * _DH, _D),
        gate_w.reshape(1, _D),
    )
    return out.reshape(_B, 1, _D)
```

```python
import jax
import jax.numpy as jnp
import numpy as np
from jax.experimental import pallas as pl
from jax.experimental.pallas import tpu as pltpu

_B = 2
_H = 32
_SK = 8192
_DH = 128
_D = 512
_NBUF = 4
_ROUNDS_PER_STEP = 6
_SHIFT = 0
_F32 = jnp.float32
_BF16 = jnp.bfloat16
_NT = (((1,), (1,)), ((), ()))
_SCALE = float(_DH) ** -0.5


def _iota(shape, dim):
    return jax.lax.broadcasted_iota(jnp.int32, shape, dim)


class _Stream:
    def __init__(self, src, dst, sem, rows, shift, lead=(), dst_lead=None, cols=None):
        self.src, self.dst, self.sem = src, dst, sem
        self.rows, self.shift, self.cols = rows, shift, cols
        self.lead = tuple(lead)
        self.dst_lead = self.lead if dst_lead is None else tuple(dst_lead)

    def _start(self, idx, prio):
        pltpu.make_async_copy(
            self.src.at[(*self.lead, *idx)], self.dst.at[(*self.dst_lead, *idx)],
            self.sem).start(priority=prio)

    def chunk(self, c, prio):
        if self.cols is not None:
            per_row = self.src.shape[-1] // self.cols
            r, col = (c // per_row) * self.rows, (c % per_row) * self.cols
            if not isinstance(c, int):
                r, col = pl.multiple_of(r, self.rows), pl.multiple_of(col, self.cols)
            self._start((pl.ds(r, self.rows), pl.ds(col, self.cols)), prio)
        elif isinstance(c, int) and c == 0:
            self._start((pl.ds(0, self.rows - self.shift),), prio)
        else:
            r = c * self.rows - self.shift
            if not isinstance(c, int):
                r = pl.multiple_of(r, 16)
            self._start((pl.ds(r, self.rows),), prio)

    def last_piece(self, prio):
        if self.shift:
            n = self.src.shape[len(self.lead)]
            self._start((pl.ds(n - self.shift, self.shift),), prio)


def _issue_rounds(a, b, lo, hi, total):
    def one_round(g):
        base = (g // 16) * 64 + g % 16
        for seg in range(4):
            a.chunk(base + seg * 16, 0)
            b.chunk(base + seg * 16, 1)

    if lo == 0 and hi > 0:
        one_round(0)
        lo = 1
    if hi - lo == 1:
        one_round(lo)
    elif hi > lo:
        def body(g, carry):
            one_round(g)
            return carry
        jax.lax.fori_loop(lo, hi, body, 0)
    if hi == total:
        a.last_piece(0)
        b.last_piece(1)


def _wait_all(buf, sem):
    pltpu.make_async_copy(buf, buf, sem).wait()


def _kernel(
    x_hbm, k_hbm, v_hbm, wq_hbm, wo_hbm,
    ckv_hbm, wbq_hbm, wuk_hbm, wuv_hbm, wbo_hbm, gate_hbm,
    out_ref,
    x_buf, gate_buf, wq_buf, wo_buf, wbq_buf, wuk_buf, wuv_buf, wbo_buf,
    ckv_buf, k_buf, v_buf, e_buf, q_buf, s_buf,
    w_sems, c_sems, k_sems, v_sems,
):
    BH = _B * _H

    cp_x = pltpu.make_async_copy(x_hbm, x_buf, w_sems.at[0])
    cp_gate = pltpu.make_async_copy(gate_hbm, gate_buf, w_sems.at[1])

    sh128 = 32 * _SHIFT
    sh512 = 16 if _SHIFT else 0

    def head_streams(i, slot):
        return (_Stream(k_hbm, k_buf, k_sems.at[slot], 128, sh128, (i,), (slot,)),
                _Stream(v_hbm, v_buf, v_sems.at[slot], 128, sh128, (i,), (slot,)))

    regions = [
        (32, _Stream(wbq_hbm, wbq_buf, w_sems.at[3], 128, sh128),
         _Stream(wuk_hbm, wuk_buf, w_sems.at[4], 128, sh128)),
        (64, _Stream(ckv_hbm, ckv_buf, c_sems.at[0], 32, 0, (0,)),
         _Stream(ckv_hbm, ckv_buf, c_sems.at[1], 32, sh512, (1,))),
        (32, _Stream(wuv_hbm, wuv_buf, w_sems.at[5], 128, sh128),
         _Stream(wbo_hbm, wbo_buf, w_sems.at[6], 32, sh512)),
        (32, _Stream(wq_hbm, wq_buf, w_sems.at[2], 16, 0, cols=1024),
         _Stream(wo_hbm, wo_buf, w_sems.at[7], 32, 0)),
    ] + [(16, *head_streams(i, i)) for i in range(_NBUF - 1)]
    state = {"region": 0, "pos": 0}

    def pump(n):
        while n > 0 and state["region"] < len(regions):
            total, sa, sb = regions[state["region"]]
            lo = state["pos"]
            hi = min(total, lo + n)
            _issue_rounds(sa, sb, lo, hi, total)
            n -= hi - lo
            state["pos"] = hi
            if hi == total:
                state["region"] += 1
                state["pos"] = 0

    def pump_until(region):
        while state["region"] < region:
            pump(regions[state["region"]][0] - state["pos"])

    step = lambda: pump(_ROUNDS_PER_STEP)

    cp_x.start()
    cp_gate.start()
    pump(8)

    for j in range(8):
        shp = (_DH, 512)
        col = _iota(shp, 1) + j * 512
        e_buf[:, j * 512:(j + 1) * 512] = jnp.where(
            (col >> 5) == _iota(shp, 0), 1.0, 0.0).astype(_BF16)

    pump_until(1)
    pump(8)

    diag = (_iota((BH, 4096), 0) & 31) == (_iota((BH, 4096), 1) & 31)
    row8 = _iota((8, _D), 0)

    cp_x.wait()
    x2 = x_buf[...].astype(_F32)
    x8 = jnp.where(row8 == 0, x2[0:1, :], jnp.where(row8 == 1, x2[1:2, :], 0.0))
    x8 = x8.astype(_BF16)

    _wait_all(wbq_buf, w_sems.at[3])
    q_b = jnp.zeros((BH, _DH), _F32)
    for t in range(4):
        xr = jnp.dot(x8[:, t * 128:(t + 1) * 128], e_buf[...],
                     preferred_element_type=_F32)
        xr = jnp.concatenate(
            [jnp.broadcast_to(xr[0:1, :], (_H, 4096)),
             jnp.broadcast_to(xr[1:2, :], (_H, 4096))], axis=0)
        lhs = jnp.where(diag, xr, 0.0).astype(_BF16)
        q_b = q_b + jnp.dot(lhs, wbq_buf[t * 4096:(t + 1) * 4096, :],
                            preferred_element_type=_F32)
        step()
    q_b = q_b.astype(_BF16)

    _wait_all(wuk_buf, w_sems.at[4])
    q_abs = []
    for t in range(4):
        r = jax.lax.dot_general(q_b, wuk_buf[t * 4096:(t + 1) * 4096, :], _NT,
                                preferred_element_type=_F32)
        r = jnp.where(diag, r, 0.0).astype(_BF16)
        q_abs.append(jax.lax.dot_general(r, e_buf[...], _NT,
                                         preferred_element_type=_F32))
        step()
    q_abs = jnp.concatenate(q_abs, axis=1).astype(_BF16)

    pump_until(2)
    pump(8)
    _wait_all(ckv_buf.at[0], c_sems.at[0])
    _wait_all(ckv_buf.at[1], c_sems.at[1])
    ctx_c = []
    KC = 2048
    for b in range(_B):
        qb = q_abs[b * _H:(b + 1) * _H, :]
        m = None
        for j in range(_SK // KC):
            s = jax.lax.dot_general(qb, ckv_buf[b, j * KC:(j + 1) * KC, :], _NT,
                                    preferred_element_type=_F32) * _SCALE
            s_buf[:, j * KC:(j + 1) * KC] = s
            mj = jnp.max(s, axis=-1, keepdims=True)
            m = mj if m is None else jnp.maximum(m, mj)
            step()
        l = jnp.zeros((_H, 1), _F32)
        cc = jnp.zeros((_H, _D), _F32)
        for j in range(_SK // KC):
            p = jnp.exp(s_buf[:, j * KC:(j + 1) * KC] - m)
            l = l + jnp.sum(p, axis=-1, keepdims=True)
            cc = cc + jnp.dot(p.astype(_BF16), ckv_buf[b, j * KC:(j + 1) * KC, :],
                              preferred_element_type=_F32)
            step()
        ctx_c.append(cc / l)
    ctx_c = jnp.concatenate(ctx_c, axis=0).astype(_BF16)

    pump_until(3)
    _wait_all(wuv_buf, w_sems.at[5])
    ctx = jnp.zeros((BH, _DH), _F32)
    for t in range(4):
        xr = jnp.dot(ctx_c[:, t * 128:(t + 1) * 128], e_buf[...],
                     preferred_element_type=_F32)
        lhs = jnp.where(diag, xr, 0.0).astype(_BF16)
        ctx = ctx + jnp.dot(lhs, wuv_buf[t * 4096:(t + 1) * 4096, :],
                            preferred_element_type=_F32)
        step()
    ctx = ctx.astype(_BF16)

    _wait_all(wbo_buf, w_sems.at[6])
    blk = (_iota((BH, 4096), 0) & 31) == (_iota((BH, 4096), 1) >> 7)
    lhs = jnp.where(blk, jnp.concatenate([ctx] * _H, axis=1), 0.0).astype(_BF16)
    t_b = jnp.dot(lhs, wbo_buf[...], preferred_element_type=_F32)
    ob0 = jnp.sum(t_b[0:_H, :], axis=0, keepdims=True)
    ob1 = jnp.sum(t_b[_H:BH, :], axis=0, keepdims=True)
    out_b = jnp.where(row8 == 0, ob0, jnp.where(row8 == 1, ob1, 0.0))
    step()

    cp_gate.wait()
    gw = gate_buf[...].astype(_F32).reshape(1, _D)
    g = jax.nn.sigmoid(jnp.sum(x8.astype(_F32) * gw, axis=-1, keepdims=True))

    pump_until(4)
    _wait_all(wq_buf, w_sems.at[2])
    q_a = jnp.dot(x8, wq_buf[...], preferred_element_type=_F32)
    q_a = q_a.astype(_BF16)
    for h in range(_H):
        q_buf[h] = q_a[:, h * _DH:(h + 1) * _DH]

    pump_until(len(regions))
    _wait_all(wo_buf, w_sems.at[7])
    row_o = _iota((8, _DH), 0)

    def body(i, acc):
        slot = i % _NBUF
        b = i // _H
        h = i % _H
        nxt = i + _NBUF - 1
        nxt_streams = head_streams(nxt, nxt % _NBUF)

        def refill(part):
            @pl.when(nxt < BH)
            def _():
                _issue_rounds(*nxt_streams, 4 * part, 4 * part + 4, 16)

        q = q_buf[h]
        refill(0)
        _wait_all(k_buf.at[slot], k_sems.at[slot])
        s = jax.lax.dot_general(q, k_buf[slot], _NT,
                                preferred_element_type=_F32) * _SCALE
        refill(1)
        m = jnp.max(s, axis=-1, keepdims=True)
        p = jnp.exp(s - m)
        l = jnp.sum(p, axis=-1, keepdims=True)
        refill(2)
        _wait_all(v_buf.at[slot], v_sems.at[slot])
        o = jnp.dot(p.astype(_BF16), v_buf[slot], preferred_element_type=_F32)
        refill(3)
        o = jnp.where(row_o == b, o / l, 0.0).astype(_BF16)
        wo_h = wo_buf[pl.ds(pl.multiple_of(h * _DH, _DH), _DH), :]
        return acc + jnp.dot(o, wo_h, preferred_element_type=_F32)

    out_a = jax.lax.fori_loop(0, BH, body, jnp.zeros((8, _D), _F32))

    res = g * out_a + (1.0 - g) * out_b
    out_ref[...] = res[0:_B, :].astype(out_ref.dtype)


@jax.jit
def pallas_gated_mix__mha_block_cached__compressed_kv_cla__decode_kernel(
    A_x: jax.Array,
    A_k_cache: jax.Array,
    A_v_cache: jax.Array,
    A_wq: jax.Array,
    A_wo: jax.Array,
    B_x: jax.Array,
    B_c_kv: jax.Array,
    B_w_q: jax.Array,
    B_w_uk: jax.Array,
    B_w_uv: jax.Array,
    B_w_o: jax.Array,
    gate_w: jax.Array,
):
    del B_x
    out_dtype = A_x.dtype
    any_spec = pl.BlockSpec(memory_space=pl.ANY)
    out = pl.pallas_call(
        _kernel,
        out_shape=jax.ShapeDtypeStruct((_B, _D), out_dtype),
        in_specs=[any_spec] * 11,
        out_specs=pl.BlockSpec(memory_space=pltpu.VMEM),
        scratch_shapes=[
            pltpu.VMEM((_B, _D), _BF16),
            pltpu.VMEM((_D,), _BF16),
            pltpu.VMEM((_D, _H * _DH), _BF16),
            pltpu.VMEM((_H * _DH, _D), _BF16),
            pltpu.VMEM((_D * _H, _DH), _BF16),
            pltpu.VMEM((_D * _H, _DH), _BF16),
            pltpu.VMEM((_D * _H, _DH), _BF16),
            pltpu.VMEM((_H * _DH, _D), _BF16),
            pltpu.VMEM((_B, _SK, _D), _BF16),
            pltpu.VMEM((_NBUF, _SK, _DH), _BF16),
            pltpu.VMEM((_NBUF, _SK, _DH), _BF16),
            pltpu.VMEM((_DH, _H * _DH), _BF16),
            pltpu.VMEM((_H, 8, _DH), _BF16),
            pltpu.VMEM((_H, _SK), _F32),
            pltpu.SemaphoreType.DMA((8,)),
            pltpu.SemaphoreType.DMA((_B,)),
            pltpu.SemaphoreType.DMA((_NBUF,)),
            pltpu.SemaphoreType.DMA((_NBUF,)),
        ],
        compiler_params=pltpu.CompilerParams(
            vmem_limit_bytes=110 * 1024 * 1024,
        ),
    )(
        A_x.reshape(_B, _D),
        A_k_cache.reshape(_B * _H, _SK, _DH),
        A_v_cache.reshape(_B * _H, _SK, _DH),
        A_wq,
        A_wo,
        B_c_kv,
        B_w_q.reshape(_D * _H, _DH),
        B_w_uk.reshape(_D * _H, _DH),
        B_w_uv.reshape(_D * _H, _DH),
        B_w_o.reshape(_H * _DH, _D),
        gate_w,
    )
    return out.reshape(_B, 1, _D)
```

```python
import jax
import jax.numpy as jnp
from jax.experimental import pallas as pl
from jax.experimental.pallas import tpu as pltpu

_B = 2
_H = 32
_SK = 8192
_DH = 128
_D = 512
_NBUF = 3
_RPS_Q = 4
_RPS_ATT = 4
_RPS_OUT = 4
_F32 = jnp.float32
_BF16 = jnp.bfloat16
_NT = (((1,), (1,)), ((), ()))
_SCALE = float(_DH) ** -0.5


def _iota(shape, dim):
    return jax.lax.broadcasted_iota(jnp.int32, shape, dim)


class _Stream:
    def __init__(self, src, dst, sem, rows, lead=(), dst_lead=None, cols=None):
        self.src, self.dst, self.sem = src, dst, sem
        self.rows, self.cols = rows, cols
        self.lead = tuple(lead)
        self.dst_lead = self.lead if dst_lead is None else tuple(dst_lead)

    def chunk(self, c, prio):
        if self.cols is None:
            r = c * self.rows
            if not isinstance(c, int):
                r = pl.multiple_of(r, self.rows)
            idx = (pl.ds(r, self.rows),)
        else:
            per_row = self.src.shape[-1] // self.cols
            r, col = (c // per_row) * self.rows, (c % per_row) * self.cols
            if not isinstance(c, int):
                r, col = pl.multiple_of(r, self.rows), pl.multiple_of(col, self.cols)
            idx = (pl.ds(r, self.rows), pl.ds(col, self.cols))
        pltpu.make_async_copy(
            self.src.at[(*self.lead, *idx)], self.dst.at[(*self.dst_lead, *idx)],
            self.sem).start(priority=prio)


def _issue_rounds(a, b, lo, hi):
    def one_round(g, carry=0):
        base = (g // 16) * 64 + g % 16
        for seg in range(4):
            a.chunk(base + seg * 16, 0)
            b.chunk(base + seg * 16, 1)
        return carry

    if hi - lo == 1:
        one_round(lo)
    elif hi > lo:
        jax.lax.fori_loop(lo, hi, one_round, 0)


def _wait_all(buf, sem):
    pltpu.make_async_copy(buf, buf, sem).wait()


def _kernel(
    x_hbm, k_hbm, v_hbm, wq_hbm, wo_hbm,
    ckv_hbm, wbq_hbm, wuk_hbm, wuv_hbm, wbo_hbm, gate_hbm,
    out_ref,
    x_buf, gate_buf, wq_buf, wo_buf, wbq_buf, wuk_buf, wuv_buf, wbo_buf,
    ckv_buf, k_buf, v_buf, e_buf, q_buf, s_buf,
    w_sems, c_sems, k_sems, v_sems, vq_sems,
):
    BH = _B * _H

    cp_x = pltpu.make_async_copy(x_hbm, x_buf, w_sems.at[0])
    cp_gate = pltpu.make_async_copy(gate_hbm, gate_buf, w_sems.at[1])

    def head_streams(i, slot):
        return (_Stream(k_hbm, k_buf, k_sems.at[slot], 128, (i,), (slot,)),
                _Stream(v_hbm, v_buf, v_sems.at[slot], 128, (i,), (slot,)))

    regions = [
        (32, _Stream(wbq_hbm, wbq_buf, w_sems.at[3], 128),
         _Stream(wuk_hbm, wuk_buf, w_sems.at[4], 128)),
        (64, _Stream(ckv_hbm, ckv_buf, c_sems.at[0], 32, (0,)),
         _Stream(ckv_hbm, ckv_buf, c_sems.at[1], 32, (1,))),
        (32, _Stream(wuv_hbm, wuv_buf, w_sems.at[5], 128),
         _Stream(wbo_hbm, wbo_buf, w_sems.at[6], 32)),
        (32, _Stream(wq_hbm, wq_buf, w_sems.at[2], 16, cols=1024),
         _Stream(wo_hbm, wo_buf, w_sems.at[7], 32)),
    ] + [(16, *head_streams(i, i)) for i in range(_NBUF - 1)]
    state = {"region": 0, "pos": 0}

    def pump(n):
        while n > 0 and state["region"] < len(regions):
            total, sa, sb = regions[state["region"]]
            lo = state["pos"]
            hi = min(total, lo + n)
            _issue_rounds(sa, sb, lo, hi)
            n -= hi - lo
            state["pos"] = hi
            if hi == total:
                state["region"] += 1
                state["pos"] = 0

    def pump_until(region):
        while state["region"] < region:
            pump(regions[state["region"]][0] - state["pos"])

    cp_x.start()
    cp_gate.start()
    pump(8)

    for j in range(8):
        shp = (_DH, 512)
        col = _iota(shp, 1) + j * 512
        e_buf[:, j * 512:(j + 1) * 512] = jnp.where(
            (col >> 5) == _iota(shp, 0), 1.0, 0.0).astype(_BF16)

    pump_until(1)
    pump(8)

    diag = (_iota((BH, 4096), 0) & 31) == (_iota((BH, 4096), 1) & 31)
    row8 = _iota((8, _D), 0)

    cp_x.wait()
    x2 = x_buf[...].astype(_F32)
    x8 = jnp.where(row8 == 0, x2[0:1, :], jnp.where(row8 == 1, x2[1:2, :], 0.0))
    x8 = x8.astype(_BF16)

    _wait_all(wbq_buf, w_sems.at[3])
    q_b = jnp.zeros((BH, _DH), _F32)
    for t in range(4):
        xr = jnp.dot(x8[:, t * 128:(t + 1) * 128], e_buf[...],
                     preferred_element_type=_F32)
        xr = jnp.concatenate(
            [jnp.broadcast_to(xr[0:1, :], (_H, 4096)),
             jnp.broadcast_to(xr[1:2, :], (_H, 4096))], axis=0)
        lhs = jnp.where(diag, xr, 0.0).astype(_BF16)
        q_b = q_b + jnp.dot(lhs, wbq_buf[t * 4096:(t + 1) * 4096, :],
                            preferred_element_type=_F32)
        pump(_RPS_Q)
    q_b = q_b.astype(_BF16)

    _wait_all(wuk_buf, w_sems.at[4])
    q_abs = []
    for t in range(4):
        r = jax.lax.dot_general(q_b, wuk_buf[t * 4096:(t + 1) * 4096, :], _NT,
                                preferred_element_type=_F32)
        r = jnp.where(diag, r, 0.0).astype(_BF16)
        q_abs.append(jax.lax.dot_general(r, e_buf[...], _NT,
                                         preferred_element_type=_F32))
        pump(_RPS_Q)
    q_abs = jnp.concatenate(q_abs, axis=1).astype(_BF16)

    pump_until(2)
    pump(8)
    _wait_all(ckv_buf.at[0], c_sems.at[0])
    _wait_all(ckv_buf.at[1], c_sems.at[1])
    ctx_c = []
    KC = 2048
    for b in range(_B):
        qb = q_abs[b * _H:(b + 1) * _H, :]
        m = None
        for j in range(_SK // KC):
            s = jax.lax.dot_general(qb, ckv_buf[b, j * KC:(j + 1) * KC, :], _NT,
                                    preferred_element_type=_F32) * _SCALE
            s_buf[:, j * KC:(j + 1) * KC] = s
            mj = jnp.max(s, axis=-1, keepdims=True)
            m = mj if m is None else jnp.maximum(m, mj)
            pump(_RPS_ATT)
        l = jnp.zeros((_H, 1), _F32)
        cc = jnp.zeros((_H, _D), _F32)
        for j in range(_SK // KC):
            p = jnp.exp(s_buf[:, j * KC:(j + 1) * KC] - m)
            l = l + jnp.sum(p, axis=-1, keepdims=True)
            cc = cc + jnp.dot(p.astype(_BF16), ckv_buf[b, j * KC:(j + 1) * KC, :],
                              preferred_element_type=_F32)
            pump(_RPS_ATT)
        ctx_c.append(cc / l)
    ctx_c = jnp.concatenate(ctx_c, axis=0).astype(_BF16)

    pump_until(4)
    _wait_all(wq_buf, w_sems.at[2])
    q_a = jnp.dot(x8, wq_buf[...], preferred_element_type=_F32)
    q_a = q_a.astype(_BF16)
    for h in range(_H):
        q_buf[h] = q_a[:, h * _DH:(h + 1) * _DH]
    pump(_RPS_OUT)

    pump_until(3)
    _wait_all(wuv_buf, w_sems.at[5])
    ctx = jnp.zeros((BH, _DH), _F32)
    for t in range(4):
        xr = jnp.dot(ctx_c[:, t * 128:(t + 1) * 128], e_buf[...],
                     preferred_element_type=_F32)
        lhs = jnp.where(diag, xr, 0.0).astype(_BF16)
        ctx = ctx + jnp.dot(lhs, wuv_buf[t * 4096:(t + 1) * 4096, :],
                            preferred_element_type=_F32)
        pump(_RPS_OUT)
    ctx = ctx.astype(_BF16)

    _wait_all(wbo_buf, w_sems.at[6])
    blk = (_iota((BH, 4096), 0) & 31) == (_iota((BH, 4096), 1) >> 7)
    lhs = jnp.where(blk, jnp.concatenate([ctx] * _H, axis=1), 0.0).astype(_BF16)
    t_b = jnp.dot(lhs, wbo_buf[...], preferred_element_type=_F32)
    ob0 = jnp.sum(t_b[0:_H, :], axis=0, keepdims=True)
    ob1 = jnp.sum(t_b[_H:BH, :], axis=0, keepdims=True)
    out_b = jnp.where(row8 == 0, ob0, jnp.where(row8 == 1, ob1, 0.0))
    pump(_RPS_OUT)

    cp_gate.wait()
    gw = gate_buf[...].astype(_F32).reshape(1, _D)
    g = jax.nn.sigmoid(jnp.sum(x8.astype(_F32) * gw, axis=-1, keepdims=True))

    pump_until(len(regions))
    _wait_all(wo_buf, w_sems.at[7])
    row_o = _iota((8, _DH), 0)

    LAST = BH - 1
    last_slot = LAST % _NBUF
    VQ = _SK // 4

    def issue_last_head(part):
        if part < 2:
            def rbody(j, carry):
                for seg in range(4):
                    r = pl.multiple_of((j + 16 * seg) * 128, 128)
                    pltpu.make_async_copy(
                        k_hbm.at[LAST, pl.ds(r, 128)],
                        k_buf.at[last_slot, pl.ds(r, 128)],
                        k_sems.at[last_slot]).start(priority=seg % 2)
                return carry
            jax.lax.fori_loop(8 * part, 8 * part + 8, rbody, 0)
        else:
            for qd in (2 * (part - 2), 2 * (part - 2) + 1):
                def rbody(j, carry, qd=qd):
                    for seg in range(2):
                        r = pl.multiple_of((2 * j + seg) * 128 + qd * VQ, 128)
                        pltpu.make_async_copy(
                            v_hbm.at[LAST, pl.ds(r, 128)],
                            v_buf.at[last_slot, pl.ds(r, 128)],
                            vq_sems.at[qd]).start(priority=seg)
                    return carry
                jax.lax.fori_loop(0, 8, rbody, 0)

    def body(i, acc, last=False):
        slot = i % _NBUF
        b = i // _H
        h = i % _H
        nxt = i + _NBUF - 1

        def refill(part):
            if last:
                return

            @pl.when(nxt < LAST)
            def _():
                _issue_rounds(*head_streams(nxt, nxt % _NBUF),
                              4 * part, 4 * part + 4)

            @pl.when(nxt == LAST)
            def _():
                issue_last_head(part)

        q = q_buf[h]
        refill(0)
        _wait_all(k_buf.at[slot], k_sems.at[slot])
        s = jax.lax.dot_general(q, k_buf[slot], _NT,
                                preferred_element_type=_F32) * _SCALE
        refill(1)
        m = jnp.max(s, axis=-1, keepdims=True)
        p = jnp.exp(s - m)
        l = jnp.sum(p, axis=-1, keepdims=True)
        p = p.astype(_BF16)
        refill(2)
        if last:
            o = jnp.zeros((8, _DH), _F32)
            for qd in range(4):
                vq = v_buf.at[slot, pl.ds(qd * VQ, VQ)]
                _wait_all(vq, vq_sems.at[qd])
                o = o + jnp.dot(p[:, qd * VQ:(qd + 1) * VQ], vq[...],
                                preferred_element_type=_F32)
        else:
            _wait_all(v_buf.at[slot], v_sems.at[slot])
            o = jnp.dot(p, v_buf[slot], preferred_element_type=_F32)
        refill(3)
        o = jnp.where(row_o == b, o / l, 0.0).astype(_BF16)
        r0 = h * _DH if last else pl.multiple_of(h * _DH, _DH)
        wo_h = wo_buf[pl.ds(r0, _DH), :]
        return acc + jnp.dot(o, wo_h, preferred_element_type=_F32)

    out_a = jax.lax.fori_loop(0, LAST, body, jnp.zeros((8, _D), _F32))
    out_a = body(LAST, out_a, last=True)

    res = g * out_a + (1.0 - g) * out_b
    out_ref[...] = res[0:_B, :].astype(out_ref.dtype)


@jax.jit
def pallas_gated_mix__mha_block_cached__compressed_kv_cla__decode_kernel(
    A_x: jax.Array,
    A_k_cache: jax.Array,
    A_v_cache: jax.Array,
    A_wq: jax.Array,
    A_wo: jax.Array,
    B_x: jax.Array,
    B_c_kv: jax.Array,
    B_w_q: jax.Array,
    B_w_uk: jax.Array,
    B_w_uv: jax.Array,
    B_w_o: jax.Array,
    gate_w: jax.Array,
):
    del B_x
    out_dtype = A_x.dtype
    any_spec = pl.BlockSpec(memory_space=pl.ANY)
    out = pl.pallas_call(
        _kernel,
        out_shape=jax.ShapeDtypeStruct((_B, _D), out_dtype),
        in_specs=[any_spec] * 11,
        out_specs=pl.BlockSpec(memory_space=pltpu.VMEM),
        scratch_shapes=[
            pltpu.VMEM((_B, _D), _BF16),
            pltpu.VMEM((_D,), _BF16),
            pltpu.VMEM((_D, _H * _DH), _BF16),
            pltpu.VMEM((_H * _DH, _D), _BF16),
            pltpu.VMEM((_D * _H, _DH), _BF16),
            pltpu.VMEM((_D * _H, _DH), _BF16),
            pltpu.VMEM((_D * _H, _DH), _BF16),
            pltpu.VMEM((_H * _DH, _D), _BF16),
            pltpu.VMEM((_B, _SK, _D), _BF16),
            pltpu.VMEM((_NBUF, _SK, _DH), _BF16),
            pltpu.VMEM((_NBUF, _SK, _DH), _BF16),
            pltpu.VMEM((_DH, _H * _DH), _BF16),
            pltpu.VMEM((_H, 8, _DH), _BF16),
            pltpu.VMEM((_H, _SK), _F32),
            pltpu.SemaphoreType.DMA((8,)),
            pltpu.SemaphoreType.DMA((_B,)),
            pltpu.SemaphoreType.DMA((_NBUF,)),
            pltpu.SemaphoreType.DMA((_NBUF,)),
            pltpu.SemaphoreType.DMA((4,)),
        ],
        compiler_params=pltpu.CompilerParams(
            vmem_limit_bytes=110 * 1024 * 1024,
        ),
    )(
        A_x.reshape(_B, _D),
        A_k_cache.reshape(_B * _H, _SK, _DH),
        A_v_cache.reshape(_B * _H, _SK, _DH),
        A_wq,
        A_wo,
        B_c_kv,
        B_w_q.reshape(_D * _H, _DH),
        B_w_uk.reshape(_D * _H, _DH),
        B_w_uv.reshape(_D * _H, _DH),
        B_w_o.reshape(_H * _DH, _D),
        gate_w,
    )
    return out.reshape(_B, 1, _D)
```
